```python
import os as _os
_os.environ.setdefault("JAX_PLATFORMS", "cpu")
import jax
import jax.numpy as jnp

def _softmax(x, axis=-1):
    return jax.nn.softmax(x, axis=axis)
def _gelu(x):
    return jax.nn.gelu(x, approximate=True)
def _silu(x):
    return jax.nn.silu(x)
def _sigmoid(x):
    return jax.nn.sigmoid(x)
def _layernorm(x, axis=-1, eps=1e-5):
    m = jnp.mean(x, axis=axis, keepdims=True)
    v = jnp.var(x, axis=axis, keepdims=True)
    return (x - m) / jnp.sqrt(v + eps)
def _scatter_add(tgt, idx, src, axis=0):
    return tgt.at[idx].add(src)
def _segment_sum(src, seg, n):
    return jax.ops.segment_sum(src, seg, n)
class _Rng:
    def __init__(self, key):
        self._k = key
    def _next(self):
        self._k, sub = jax.random.split(self._k)
        return sub
    def normal(self, shape):
        return jax.random.normal(self._next(), shape, dtype=jnp.bfloat16)
    def randint(self, lo, hi, shape):
        return jax.random.randint(self._next(), shape, lo, hi, dtype=jnp.int32)
    def uniform(self, shape, lo=0.0, hi=1.0):
        return jax.random.uniform(self._next(), shape, jnp.bfloat16, lo, hi)
    def permutation(self, n):
        return jax.random.permutation(self._next(), n)


kernel_name = 'concat_heads__gqa_block_cached__sliding_block_cached__decode'

def setup_inputs():
    _rng = _Rng(jax.random.key(int.from_bytes(__import__("os").urandom(4), "little")))
    _w = (lambda a: (lambda t: t.astype(jnp.bfloat16) if jnp.issubdtype(t.dtype, jnp.floating) else t)(jnp.asarray(a)))
    def _A_setup():
        B, Sq, D = 1, 1, 576
        Hq, Hkv, Sk, Dh = 32, 16, 8192, 128
        assert Hq % Hkv == 0, (Hq, Hkv)
        return {
            "x": _w((lambda *s: _rng.normal(s) * 0.8)(B, Sq, D)),
            "k_cache": _w((lambda *s: _rng.normal(s) * 0.8)(B, Hkv, Sk, Dh)),
            "v_cache": _w((lambda *s: _rng.normal(s) * 0.05)(B, Hkv, Sk, Dh)),
            "wq": _w((lambda *s: _rng.normal(s) * 0.8)(D, Hq * Dh) * (D ** -0.5)),
            "wo": _w((lambda *s: _rng.normal(s) * 0.05)(Hq * Dh, D) * ((Hq * Dh) ** -0.5)),
        }
    _A_in = _A_setup()

    def _B_setup():
        B, Sq, D = 1, 1, 576
        Hq, Hkv, Sk, Dh = 32, 16, 8192, 128
        assert Hq % Hkv == 0, (Hq, Hkv)
        return {
            "x": _w((lambda *s: _rng.normal(s) * 0.8)(B, Sq, D)),
            "k_cache": _w((lambda *s: _rng.normal(s) * 0.8)(B, Hkv, Sk, Dh)),
            "v_cache": _w((lambda *s: _rng.normal(s) * 0.05)(B, Hkv, Sk, Dh)),
            "wq": _w((lambda *s: _rng.normal(s) * 0.8)(D, Hq * Dh) * (D ** -0.5)),
            "wo": _w((lambda *s: _rng.normal(s) * 0.05)(Hq * Dh, D) * ((Hq * Dh) ** -0.5)),
        }
    _B_in = _B_setup()

    return {
        "A_x": _A_in["x"],
        "A_k_cache": _A_in["k_cache"],
        "A_v_cache": _A_in["v_cache"],
        "A_wq": _A_in["wq"],
        "A_wo": _A_in["wo"],
        "B_x": _B_in["x"],
        "B_k_cache": _B_in["k_cache"],
        "B_v_cache": _B_in["v_cache"],
        "B_wq": _B_in["wq"],
        "B_wo": _B_in["wo"],
    }

def reference(A_x, A_k_cache, A_v_cache, A_wq, A_wo, B_x, B_k_cache, B_v_cache, B_wq, B_wo):
    def _A_ref(x, k_cache, v_cache, wq, wo):
        B, Sq, D = x.shape
        Hq, Dh = 32, 128
        Hkv = k_cache.shape[1]
        rep = Hq // Hkv
        q = (lambda x, *d: x.transpose(*d))((x @ wq).reshape(B, Sq, Hq, Dh), 0, 2, 1, 3)
        k = jnp.repeat(k_cache, rep, axis=1)
        v = jnp.repeat(v_cache, rep, axis=1)
        scores = jnp.einsum("bhqd,bhkd->bhqk", q, k) * (Dh ** -0.5)
        p = _softmax(scores, axis=-1)
        o = jnp.einsum("bhqk,bhkd->bhqd", p, v)
        return (lambda x, *d: x.transpose(*d))(o, 0, 2, 1, 3).reshape(B, Sq, Hq * Dh) @ wo

    def _B_ref(x, k_cache, v_cache, wq, wo):
        B, Sq, D = x.shape
        Hq, Dh = 32, 128
        Hkv, Sk = k_cache.shape[1], k_cache.shape[2]
        W = min(4096, max(256, Sk // 4))
        rep = Hq // Hkv
        q = (lambda x, *d: x.transpose(*d))((x @ wq).reshape(B, Sq, Hq, Dh), 0, 2, 1, 3)
        k = jnp.repeat(k_cache[:, :, Sk - W:, :], rep, axis=1)
        v = jnp.repeat(v_cache[:, :, Sk - W:, :], rep, axis=1)
        scores = jnp.einsum("bhqd,bhkd->bhqk", q, k) * (Dh ** -0.5)
        p = _softmax(scores, axis=-1)
        o = jnp.einsum("bhqk,bhkd->bhqd", p, v)
        return (lambda x, *d: x.transpose(*d))(o, 0, 2, 1, 3).reshape(B, Sq, Hq * Dh) @ wo

    a = _A_ref(A_x, A_k_cache, A_v_cache, A_wq, A_wo)
    b = _B_ref(B_x, B_k_cache, B_v_cache, B_wq, B_wo)
    return jnp.concatenate([a, b], axis=-1)
```

```python
import jax
import jax.numpy as jnp
from jax import lax
import jax.experimental.pallas as pl
import jax.experimental.pallas.tpu as pltpu

_NT = (((1,), (1,)), ((), ()))


@jax.jit
def pallas_concat_heads__gqa_block_cached__sliding_block_cached__decode_kernel(
    A_x, A_k_cache, A_v_cache, A_wq, A_wo, B_x, B_k_cache, B_v_cache, B_wq, B_wo,
):
    bf16, f32 = jnp.bfloat16, jnp.float32
    D, HQ, HKV, SK, DH = 576, 32, 16, 8192, 128
    W = min(4096, max(256, SK // 4))
    scale = DH ** -0.5
    kchunk = 2048
    ka_groups = (8, 8)
    va_groups = (8, 4, 2, 1, 1)
    wo_cols = (2048, 1024, 512, 256, 256)

    def kern(xa_h, ka_h, va_h, wqa_h, woa_h, xb_h, kb_h, vb_h, wqb_h, wob_h, out_ref,
             xa, xb, wqa, wqb, ka, va, kb, vb, woa, wob, q_s, s_s, pa_s, pb_s, l_s, oa_s, ob_s, sems):
        n = [0]

        def copy(src, dst):
            c = pltpu.make_async_copy(src, dst, sems.at[n[0]])
            n[0] += 1
            c.start()
            return c

        c_wqb = copy(wqb_h, wqb)
        c_xb = copy(xb_h, xb)
        c_xa = copy(xa_h, xa)
        c_wqa = copy(wqa_h, wqa)
        c_kb = copy(kb_h.at[:, pl.ds(SK - W, W), :], kb)
        c_vb = copy(vb_h.at[:, pl.ds(SK - W, W), :], vb)
        c_wob = copy(wob_h, wob)
        c_ka, h0 = [], 0
        for g in ka_groups:
            c_ka.append((copy(ka_h.at[pl.ds(h0, g)], ka.at[pl.ds(h0, g)]), h0, g))
            h0 += g
        c_va, h0 = [], 0
        for g in va_groups:
            c_va.append((copy(va_h.at[pl.ds(h0, g)], va.at[pl.ds(h0, g)]), h0, g))
            h0 += g
        c_woa, k0 = [], 0
        for g in wo_cols:
            c_woa.append((copy(woa_h.at[:, pl.ds(k0, g)], woa.at[:, pl.ds(k0, g)]), k0, g))
            k0 += g

        row = lax.broadcasted_iota(jnp.int32, (8, DH), 0)

        def qproj(x_ref, wq_ref, base):
            x8 = jnp.broadcast_to(x_ref[...], (8, D))

            def body(h, carry):
                w = wq_ref[:, pl.ds(pl.multiple_of(h * 2 * DH, 2 * DH), 2 * DH)]
                q = jnp.dot(x8, w, preferred_element_type=f32)
                q_s[base + h] = jnp.where(row == 0, q[:, :DH], q[:, DH:])
                return carry
            lax.fori_loop(0, HKV, body, None)

        def scores(k_ref, p_ref, base, h0, nh, sk):
            def body(h, carry):
                q = q_s[base + h].astype(bf16)

                def inner(c, m):
                    off = pl.multiple_of(c * kchunk, kchunk)
                    s = lax.dot_general(q, k_ref[h, pl.ds(off, kchunk), :], _NT, preferred_element_type=f32) * scale
                    s_s[:, pl.ds(off, kchunk)] = s
                    for j in range(kchunk // 128):
                        m = jnp.maximum(m, s[:, j * 128:(j + 1) * 128])
                    return m
                m = lax.fori_loop(0, sk // kchunk, inner, jnp.full((8, 128), -jnp.inf, f32))
                m = jnp.max(m, axis=1, keepdims=True)

                def inner2(c, l):
                    off = pl.multiple_of(c * kchunk, kchunk)
                    p = jnp.exp(s_s[:, pl.ds(off, kchunk)] - m)
                    p_ref[h, :, pl.ds(off, kchunk)] = p
                    for j in range(kchunk // 128):
                        l = l + p[:, j * 128:(j + 1) * 128]
                    return l
                l = lax.fori_loop(0, sk // kchunk, inner2, jnp.zeros((8, 128), f32))
                l = jnp.sum(l, axis=1, keepdims=True)
                l_s[base + h] = jnp.broadcast_to(1.0 / l, (8, DH))
                return carry
            lax.fori_loop(h0, h0 + nh, body, None)

        def pv(v_ref, p_ref, o_ref, base, h0, nh, sk):
            def body(h, carry):
                def inner(c, acc):
                    off = pl.multiple_of(c * kchunk, kchunk)
                    p = p_ref[h, :, pl.ds(off, kchunk)].astype(bf16)
                    return acc + jnp.dot(p, v_ref[h, pl.ds(off, kchunk), :], preferred_element_type=f32)
                acc = lax.fori_loop(0, sk // kchunk, inner, jnp.zeros((8, DH), f32))
                o = acc * l_s[base + h]
                off = pl.multiple_of(h * 2 * DH, 2 * DH)
                o_ref[:, pl.ds(off, 2 * DH)] = jnp.concatenate(
                    [jnp.broadcast_to(o[0:1], (8, DH)), jnp.broadcast_to(o[1:2], (8, DH))], axis=1)
                return carry
            lax.fori_loop(h0, h0 + nh, body, None)

        def oproj(o_ref, wo_ref, k0, nk, acc, step=512):
            step = min(step, nk)

            def body(i, acc):
                off = pl.multiple_of(k0 + i * step, step)
                o = o_ref[:, pl.ds(off, step)].astype(bf16)
                return acc + lax.dot_general(o, wo_ref[:, pl.ds(off, step)], _NT, preferred_element_type=f32)
            if nk == step:
                return body(0, acc)
            return lax.fori_loop(0, nk // step, body, acc)

        c_wqb.wait()
        c_xb.wait()
        qproj(xb, wqb, HKV)
        c_xa.wait()
        c_wqa.wait()
        qproj(xa, wqa, 0)
        c_kb.wait()
        scores(kb, pb_s, HKV, 0, HKV, W)
        c_vb.wait()
        pv(vb, pb_s, ob_s, HKV, 0, HKV, W)
        c_wob.wait()
        out_b = oproj(ob_s, wob, 0, HQ * DH, jnp.zeros((8, D), f32))
        for c, h0, g in c_ka:
            c.wait()
            scores(ka, pa_s, 0, h0, g, SK)
        for c, h0, g in c_va:
            c.wait()
            pv(va, pa_s, oa_s, 0, h0, g, SK)
        acc = jnp.zeros((8, D), f32)
        for c, k0, g in c_woa:
            c.wait()
            acc = oproj(oa_s, woa, k0, g, acc)
        out_ref[...] = jnp.concatenate([acc[0:1], out_b[0:1]], axis=1).astype(out_ref.dtype)

    nsem = 7 + len(ka_groups) + len(va_groups) + len(wo_cols)
    out = pl.pallas_call(
        kern,
        out_shape=jax.ShapeDtypeStruct((1, 2 * D), bf16),
        in_specs=[pl.BlockSpec(memory_space=pltpu.HBM)] * 10,
        out_specs=pl.BlockSpec(memory_space=pltpu.VMEM),
        scratch_shapes=[
            pltpu.VMEM((1, D), bf16), pltpu.VMEM((1, D), bf16),
            pltpu.VMEM((D, HQ * DH), bf16), pltpu.VMEM((D, HQ * DH), bf16),
            pltpu.VMEM((HKV, SK, DH), bf16), pltpu.VMEM((HKV, SK, DH), bf16),
            pltpu.VMEM((HKV, W, DH), bf16), pltpu.VMEM((HKV, W, DH), bf16),
            pltpu.VMEM((D, HQ * DH), bf16), pltpu.VMEM((D, HQ * DH), bf16),
            pltpu.VMEM((2 * HKV, 8, DH), f32),
            pltpu.VMEM((8, SK), f32),
            pltpu.VMEM((HKV, 8, SK), f32), pltpu.VMEM((HKV, 8, W), f32),
            pltpu.VMEM((2 * HKV, 8, DH), f32),
            pltpu.VMEM((8, HQ * DH), f32), pltpu.VMEM((8, HQ * DH), f32),
            pltpu.SemaphoreType.DMA((nsem,)),
        ],
        compiler_params=pltpu.CompilerParams(vmem_limit_bytes=120 * 1024 * 1024),
    )(A_x.reshape(1, D), A_k_cache.reshape(HKV, SK, DH), A_v_cache.reshape(HKV, SK, DH), A_wq, A_wo.T,
      B_x.reshape(1, D), B_k_cache.reshape(HKV, SK, DH), B_v_cache.reshape(HKV, SK, DH), B_wq, B_wo.T)
    return out.reshape(1, 1, 2 * D)
```

```python
import functools

import jax
import jax.numpy as jnp
from jax import lax
import jax.experimental.pallas as pl
import jax.experimental.pallas.tpu as pltpu

HQ, DH = 32, 128
_NT = (((1,), (1,)), ((), ()))

_KV_CHUNK = 2048
_PIECE = 16
_N_PIECES = 24
_N_STAGE = 4
_AHEAD = 2
_WOB_ROWS = (320, 128, 128)
_TAIL_ROWS = 128
_TAIL_COLS = (2560, 1024, 512)
_N_SEMS = 9 + len(_WOB_ROWS) + len(_TAIL_COLS)


def _body(xa_h, ka_h, va_h, wqa_h, woa_h, xb_h, kb_h, vb_h, wqb_h, wob_h, out_ref,
          xa, xb, wqa, wqb, ka, va, kb, vb, woa, wob,
          q_s, s_s, pa_s, pb_s, l_s, oa_s, ob_s, acc_s, stage,
          sems, in_sems, out_sems):
    f32, bf16 = jnp.float32, jnp.bfloat16
    hkv, sk, _ = ka.shape
    win = kb.shape[1]
    d = wqa.shape[0]
    n_pairs = hkv // 2
    scale = DH ** -0.5
    relay_row0 = d - _PIECE * _N_PIECES
    lag = _N_STAGE - _AHEAD

    next_sem = iter(range(_N_SEMS))

    def copy(src, dst):
        return pltpu.make_async_copy(src, dst, sems.at[next(next_sem)])

    def pair(src, dst, sem0, j):
        heads = pl.ds(2 * j, 2)
        return pltpu.make_async_copy(src.at[heads], dst.at[heads], sems.at[sem0 + j])

    ka_pair = functools.partial(pair, ka_h, ka, _N_SEMS)
    va_pair = functools.partial(pair, va_h, va, _N_SEMS + n_pairs)

    def window(src, dst, h0):
        heads = pl.ds(h0, n_pairs)
        return copy(src.at[heads, pl.ds(sk - win, win), :], dst.at[heads])

    def block(src, dst, *idx):
        return copy(src.at[idx], dst.at[idx])

    c_wqa, c_xa, c_xb, c_wqb = copy(wqa_h, wqa), copy(xa_h, xa), copy(xb_h, xb), copy(wqb_h, wqb)
    c_kb = [window(kb_h, kb, h0) for h0 in (0, n_pairs)]
    c_vb = [window(vb_h, vb, h0) for h0 in (0, n_pairs)]
    c_mid = block(woa_h, woa, pl.ds(_TAIL_ROWS, relay_row0 - _TAIL_ROWS))
    c_wob, r0 = [], 0
    for n in _WOB_ROWS:
        c_wob.append((block(wob_h, wob, pl.ds(r0, n)), r0, n))
        r0 += n
    c_tail, k0 = [], 0
    for n in _TAIL_COLS:
        c_tail.append((block(woa_h, woa, pl.ds(0, _TAIL_ROWS), pl.ds(k0, n)), k0, n))
        k0 += n

    def piece(i):
        return pl.ds(pl.multiple_of(relay_row0 + i * _PIECE, _PIECE), _PIECE)

    def slot(i):
        return i & (_N_STAGE - 1)

    def relay_in(i):
        return pltpu.make_async_copy(woa_h.at[piece(i)], stage.at[slot(i)], in_sems.at[slot(i)])

    def relay_out(i):
        return pltpu.make_async_copy(stage.at[slot(i)], woa.at[piece(i)], out_sems.at[slot(i)])

    def relay(i):
        static = isinstance(i, int)
        relay_in(i).wait()
        relay_out(i).start()
        if not static or i >= lag:
            relay_out(i - lag).wait()
        if not static or i + _AHEAD < _N_PIECES:
            relay_in(i + _AHEAD).start()

    row = lax.broadcasted_iota(jnp.int32, (8, DH), 0)

    def q_proj(x_ref, wq_ref, base):
        x8 = jnp.broadcast_to(x_ref[...], (8, d))

        @pl.loop(0, hkv)
        def _(h):
            w = wq_ref[:, pl.ds(pl.multiple_of(h * 2 * DH, 2 * DH), 2 * DH)]
            q = jnp.dot(x8, w, preferred_element_type=f32)
            q_s[base + h] = jnp.where(row == 0, q[:, :DH], q[:, DH:])

    def fold(op, acc, x):
        for j in range(x.shape[1] // 128):
            acc = op(acc, x[:, j * 128:(j + 1) * 128])
        return acc

    def chunk(c):
        return pl.ds(pl.multiple_of(c * _KV_CHUNK, _KV_CHUNK), _KV_CHUNK)

    def softmax(k_ref, p_ref, base, h0, nh):
        n_chunks = k_ref.shape[1] // _KV_CHUNK

        @pl.loop(0, nh)
        def _(i):
            h = h0 + i
            q = q_s[base + h].astype(bf16)

            def scores(c, m):
                s = lax.dot_general(q, k_ref[h, chunk(c), :], _NT, preferred_element_type=f32) * scale
                s_s[:, chunk(c)] = s
                return fold(jnp.maximum, m, s)

            m = lax.fori_loop(0, n_chunks, scores, jnp.full((8, 128), -jnp.inf, f32))
            m = jnp.max(m, axis=1, keepdims=True)

            def exps(c, l):
                p = jnp.exp(s_s[:, chunk(c)] - m)
                p_ref[h, :, chunk(c)] = p
                return fold(jnp.add, l, p)

            l = lax.fori_loop(0, n_chunks, exps, jnp.zeros((8, 128), f32))
            l_s[base + h] = jnp.broadcast_to(jnp.sum(l, axis=1, keepdims=True), (8, DH))

    def weighted_v(v_ref, p_ref, o_ref, base, h0, nh):
        n_chunks = v_ref.shape[1] // _KV_CHUNK

        @pl.loop(0, nh)
        def _(i):
            h = h0 + i

            def step(c, acc):
                p = p_ref[h, :, chunk(c)].astype(bf16)
                return acc + jnp.dot(p, v_ref[h, chunk(c), :], preferred_element_type=f32)

            o = lax.fori_loop(0, n_chunks, step, jnp.zeros((8, DH), f32)) / l_s[base + h]
            o_ref[:, pl.ds(pl.multiple_of(h * 2 * DH, 2 * DH), 2 * DH)] = jnp.concatenate(
                [jnp.broadcast_to(o[0:1], (8, DH)), jnp.broadcast_to(o[1:2], (8, DH))], axis=1)

    def o_dot(o_ref, wo_ref, rows, cols):
        return lax.dot_general(o_ref[:, cols].astype(bf16), wo_ref[rows, cols], _NT,
                               preferred_element_type=f32)

    def out_proj(o_ref, wo_ref, r0, n, lane0):
        rows = pl.ds(r0, n)
        if n <= 128:
            res = o_dot(o_ref, wo_ref, rows, pl.ds(0, HQ * DH))
        else:
            res = lax.fori_loop(0, HQ * DH // _KV_CHUNK,
                                lambda c, acc: acc + o_dot(o_ref, wo_ref, rows, chunk(c)),
                                jnp.zeros((8, n), f32))
        out_ref[:, lane0 + r0:lane0 + r0 + n] = res[0:1].astype(out_ref.dtype)

    c_wqa.start()
    for i in range(_AHEAD):
        relay_in(i).start()
    c_xa.start()
    c_xb.start()
    c_wqb.start()
    for j in range(n_pairs):
        ka_pair(j).start()

    relay(0)
    relay(1)
    c_wqa.wait()
    c_xa.wait()
    q_proj(xa, wqa, 0)
    relay(2)
    c_xb.wait()
    c_wqb.wait()
    q_proj(xb, wqb, hkv)

    @pl.loop(0, n_pairs)
    def _(j):
        relay(3 + j)
        ka_pair(j).wait()
        va_pair(j).start()
        softmax(ka, pa_s, 0, 2 * j, 2)

    for c in c_kb + c_vb:
        c.start()

    @pl.loop(0, n_pairs)
    def _(j):
        relay(3 + n_pairs + j)
        va_pair(j).wait()
        weighted_v(va, pa_s, oa_s, 0, 2 * j, 2)

    for c in [c_mid] + [c[0] for c in c_wob + c_tail]:
        c.start()

    for j in range(2):
        relay(3 + hkv + j)
        c_kb[j].wait()
        softmax(kb, pb_s, hkv, n_pairs * j, n_pairs)
    for j in range(2):
        relay(5 + hkv + j)
        c_vb[j].wait()
        weighted_v(vb, pb_s, ob_s, hkv, n_pairs * j, n_pairs)

    late_row0 = d // 128 * 128
    assert relay_row0 + (7 + hkv - lag) * _PIECE >= late_row0
    c_mid.wait()
    out_proj(oa_s, woa, _TAIL_ROWS, late_row0 - _TAIL_ROWS, 0)
    for i in range(7 + hkv, _N_PIECES):
        relay(i)
    for c, r0, n in c_wob[:-1]:
        c.wait()
        out_proj(ob_s, wob, r0, n, d)
    for i in range(_N_PIECES - lag, _N_PIECES):
        relay_out(i).wait()
    out_proj(oa_s, woa, late_row0, d - late_row0, 0)
    c, r0, n = c_wob[-1]
    c.wait()
    out_proj(ob_s, wob, r0, n, d)

    acc_s[...] = jnp.zeros(acc_s.shape, f32)
    for c, k0, n in c_tail[:-1]:
        c.wait()
        acc_s[...] = acc_s[...] + o_dot(oa_s, woa, pl.ds(0, _TAIL_ROWS), pl.ds(k0, n))
    c, k0, n = c_tail[-1]
    c.wait()
    res = acc_s[...] + o_dot(oa_s, woa, pl.ds(0, _TAIL_ROWS), pl.ds(k0, n))
    out_ref[:, 0:_TAIL_ROWS] = res[0:1].astype(out_ref.dtype)


@jax.jit
def pallas_concat_heads__gqa_block_cached__sliding_block_cached__decode_kernel(
    A_x: jax.Array,
    A_k_cache: jax.Array,
    A_v_cache: jax.Array,
    A_wq: jax.Array,
    A_wo: jax.Array,
    B_x: jax.Array,
    B_k_cache: jax.Array,
    B_v_cache: jax.Array,
    B_wq: jax.Array,
    B_wo: jax.Array,
):
    _, hkv, sk, _ = A_k_cache.shape
    d = A_x.shape[-1]
    win = min(4096, max(256, sk // 4))
    assert A_x.shape == (1, 1, d) and HQ == 2 * hkv
    dt, f32 = A_x.dtype, jnp.float32

    def kernel(*refs):
        pl.run_scoped(
            functools.partial(_body, *refs),
            pltpu.SemaphoreType.DMA((_N_SEMS + hkv,)),
            pltpu.SemaphoreType.DMA((_N_STAGE,)),
            pltpu.SemaphoreType.DMA((_N_STAGE,)),
        )

    x_buf = pltpu.VMEM((1, d), dt)
    w_buf = pltpu.VMEM((d, HQ * DH), dt)
    a_buf = pltpu.VMEM((hkv, sk, DH), dt)
    b_buf = pltpu.VMEM((hkv, win, DH), dt)
    out = pl.pallas_call(
        kernel,
        out_shape=jax.ShapeDtypeStruct((1, 2 * d), dt),
        in_specs=[pl.BlockSpec(memory_space=pltpu.HBM)] * 10,
        out_specs=pl.BlockSpec(memory_space=pltpu.VMEM),
        scratch_shapes=[
            x_buf, x_buf, w_buf, w_buf, a_buf, a_buf, b_buf, b_buf, w_buf, w_buf,
            pltpu.VMEM((2 * hkv, 8, DH), f32),
            pltpu.VMEM((8, sk), f32),
            pltpu.VMEM((hkv, 8, sk), f32),
            pltpu.VMEM((hkv, 8, win), f32),
            pltpu.VMEM((2 * hkv, 8, DH), f32),
            pltpu.VMEM((8, HQ * DH), f32),
            pltpu.VMEM((8, HQ * DH), f32),
            pltpu.VMEM((8, _TAIL_ROWS), f32),
            pltpu.SMEM((_N_STAGE, _PIECE, HQ * DH), dt),
        ],
        compiler_params=pltpu.CompilerParams(vmem_limit_bytes=120 * 1024 * 1024),
    )(
        A_x.reshape(1, d), A_k_cache.reshape(hkv, sk, DH), A_v_cache.reshape(hkv, sk, DH), A_wq, A_wo.T,
        B_x.reshape(1, d), B_k_cache.reshape(hkv, sk, DH), B_v_cache.reshape(hkv, sk, DH), B_wq, B_wo.T,
    )
    return out.reshape(1, 1, 2 * d)
```

```python
import functools

import jax
import jax.numpy as jnp
from jax import lax
import jax.experimental.pallas as pl
import jax.experimental.pallas.tpu as pltpu

HQ, DH = 32, 128
E = HQ * DH
_NT = (((1,), (1,)), ((), ()))

_RUN = 128
_CHUNK = 256
_LOOKAHEAD = 8
_W_RUN = (8, 2048)
_W_GROUP = 64
_WOB_SPLIT = 5
_N_PIECES = 95
_N_STAGE = 4
_AHEAD = 2
_N_PRE = 10
_TAIL_ROWS = 128
_TAIL_COLS = (1536, 1024, 1024, 512)
_N_SEMS = 9 + len(_TAIL_COLS)


def _ds(start, size, align):
    if not isinstance(start, int):
        start = pl.multiple_of(start, align)
    return pl.ds(start, size)


def _fold(op, acc, x):
    for j in range(x.shape[1] // 128):
        acc = op(acc, x[:, j * 128:(j + 1) * 128])
    return acc


def _unrolled_loop(n, unroll):
    def run(fn):
        @pl.loop(0, n // unroll)
        def _(g):
            for i in range(unroll):
                fn(g * unroll + i)
    return run


def _body(xa_h, ka_h, va_h, wqa_h, woa_h, xb_h, kb_h, vb_h, wqb_h, wob_h, out_ref,
          x_s, wq, kv, woa, wob, q_s, s_s, m_s, l_s, o_s, att, acc_s, stage,
          sems, in_sems, out_sems):
    f32, bf16 = jnp.float32, jnp.bfloat16
    hkv, sk, _ = ka_h.shape
    d = woa.shape[0]
    n_k = kv.shape[0] // 2
    n_a = sk // _CHUNK
    win0 = sk - (n_k - n_a) * _CHUNK
    scale = DH ** -0.5

    next_sem = iter(range(2 * n_k, 2 * n_k + _N_SEMS))

    def blocks(src, dst, indices):
        sem = sems.at[next(next_sem)]
        return [pltpu.make_async_copy(src.at[ix], dst.at[ix], sem) for ix in indices]

    def slabs(src, dst, groups, c0, c1):
        return blocks(src, dst, [(groups, pl.ds(r, _W_RUN[0]), pl.ds(c, _W_RUN[1]))
                                 for c in range(c0, c1, _W_RUN[1])
                                 for r in range(0, _W_GROUP, _W_RUN[0])])

    def start(copies):
        for c in copies:
            c.start()

    def wait(copies):
        for c in copies:
            c.wait()

    caches = ((0, n_a, ka_h, 0), (n_a, n_k, kb_h, win0),
              (n_k, n_k + n_a, va_h, 0), (n_k + n_a, 2 * n_k, vb_h, win0))

    def kv_start(j, candidates):
        for lo, hi, src, row0 in candidates:
            @pl.when((j >= lo) & (j < hi))
            def _():
                for r in range(0, _CHUNK, _RUN):
                    rows = _ds(row0 + (j - lo) * _CHUNK + r, _RUN, _RUN)
                    pltpu.make_async_copy(src.at[:, rows], kv.at[j, :, pl.ds(r, _RUN)], sems.at[j]).start()

    def kv_wait(j):
        pltpu.make_async_copy(kv.at[j], kv.at[j], sems.at[j]).wait()

    lag = _N_STAGE - _AHEAD

    def piece(i):
        return (_ds(d - _W_RUN[0] - (i >> 1) * _W_RUN[0], _W_RUN[0], _W_RUN[0]),
                _ds((i & 1) * _W_RUN[1], _W_RUN[1], _W_RUN[1]))

    def relay_in(i):
        slot = i & (_N_STAGE - 1)
        return pltpu.make_async_copy(woa_h.at[piece(i)], stage.at[slot], in_sems.at[slot])

    def relay_out(i):
        slot = i & (_N_STAGE - 1)
        return pltpu.make_async_copy(stage.at[slot], woa.at[piece(i)], out_sems.at[slot])

    def relay(i):
        traced = not isinstance(i, int)
        relay_in(i).wait()
        relay_out(i).start()
        if traced or i >= lag:
            relay_out(i - lag).wait()
        if traced or i + _AHEAD < _N_PIECES:
            relay_in(i + _AHEAD).start()

    assert lag <= _N_PRE - _LOOKAHEAD and _N_PRE + 2 * n_k + _AHEAD <= _N_PIECES

    n_groups = d // _W_GROUP
    every, low, high = pl.ds(0, n_groups), pl.ds(0, _WOB_SPLIT), pl.ds(_WOB_SPLIT, n_groups - _WOB_SPLIT)
    c_wqa = slabs(wqa_h, wq.at[0], every, 0, E)
    c_wqb = slabs(wqb_h, wq.at[1], every, 0, E)
    c_x = [pltpu.make_async_copy(src, x_s.at[b], sems.at[next(next_sem)]) for b, src in enumerate((xa_h, xb_h))]
    c_wob = [slabs(wob_h, wob, low, 0, E), slabs(wob_h, wob, high, 0, E // 2), slabs(wob_h, wob, high, E // 2, E)]
    relayed_row0 = d - (_N_PIECES + 1) // 2 * _W_RUN[0]
    c_mid = blocks(woa_h, woa, [piece(_N_PIECES)] * (_N_PIECES % 2)
                   + [pl.ds(_TAIL_ROWS, relayed_row0 - _TAIL_ROWS)])
    tail_cols = [pl.ds(sum(_TAIL_COLS[:i]), n) for i, n in enumerate(_TAIL_COLS)]
    c_tail = [blocks(woa_h, woa, [(pl.ds(0, _TAIL_ROWS), cols)]) for cols in tail_cols]

    def q_proj(b, h0, n):
        x8 = jnp.broadcast_to(x_s[b], (8, d))
        row = lax.broadcasted_iota(jnp.int32, (8, DH), 0)

        @_unrolled_loop(n, 2)
        def _(i):
            h = h0 + i
            w = wq[b, :, :, _ds(h * 2 * DH, 2 * DH, 2 * DH)].reshape(d, 2 * DH)
            q = jnp.dot(x8, w, preferred_element_type=f32)
            q_s[b * hkv + h] = jnp.where(row == 0, q[:, :DH], q[:, DH:])

    def out_dot(b, w, cols):
        return lax.dot_general(att[b, :, cols].astype(bf16), w, _NT, preferred_element_type=f32)

    def out_proj(b, weights, acc, c0, c1, step=1024):
        def add(i, acc):
            cols = _ds(c0 + i * step, step, step)
            return acc + out_dot(b, weights(cols).reshape(acc.shape[1], step), cols)
        return lax.fori_loop(0, (c1 - c0) // step, add, acc)

    def emit(lane0, res):
        out_ref[:, lane0:lane0 + res.shape[1]] = res[0:1].astype(out_ref.dtype)

    start(c_wqa)
    for i in range(_AHEAD):
        relay_in(i).start()
    start(c_x)
    for i in range(lag):
        relay(i)
    start(c_wqb)
    m_s[...] = jnp.full(m_s.shape, -jnp.inf, f32)
    l_s[...] = jnp.zeros(l_s.shape, f32)
    o_s[...] = jnp.zeros(o_s.shape, f32)

    @pl.loop(lag, _N_PRE)
    def _(i):
        relay(i)
        kv_start(i + _LOOKAHEAD - _N_PRE, caches[:1])

        @pl.when(i == _N_PRE - 2)
        def _():
            wait(c_wqa)
            wait(c_x)

        @pl.when(i >= _N_PRE - 2)
        def _():
            q_proj(0, (i - _N_PRE + 2) * (hkv // 2), hkv // 2)

    @pl.loop(0, n_k)
    def _(j):
        kv_start(j + _LOOKAHEAD, caches[:3])
        relay(_N_PRE + j)

        @pl.when(j == 0)
        def _():
            wait(c_wqb)

        @pl.when(j < 2)
        def _():
            q_proj(1, j * (hkv // 2), hkv // 2)

        kv_wait(j)
        base = jnp.where(j < n_a, 0, hkv)

        @_unrolled_loop(hkv, 8)
        def _(h):
            s = lax.dot_general(q_s[base + h].astype(bf16), kv[j, h], _NT, preferred_element_type=f32) * scale
            s_s[j, h] = s
            m_s[base + h] = _fold(jnp.maximum, m_s[base + h], s)

    @_unrolled_loop(2 * hkv, 16)
    def _(i):
        m_s[i] = jnp.broadcast_to(jnp.max(m_s[i], axis=1, keepdims=True), (8, 128))

    @pl.loop(0, n_k)
    def _(j):
        kv_start(n_k + j + _LOOKAHEAD, caches[2:])

        @pl.when(j == n_k - 5)
        def _():
            start(c_wob[0])

        @pl.when(j == n_k - 2)
        def _():
            start(c_wob[1])

        relay(_N_PRE + n_k + j)
        kv_wait(n_k + j)
        base = jnp.where(j < n_a, 0, hkv)

        @_unrolled_loop(hkv, 8)
        def _(h):
            p = jnp.exp(s_s[j, h] - jnp.concatenate([m_s[base + h]] * (_CHUNK // 128), axis=1))
            l_s[base + h] = _fold(jnp.add, l_s[base + h], p)
            o_s[base + h] = o_s[base + h] + jnp.dot(p.astype(bf16), kv[n_k + j, h], preferred_element_type=f32)

    for copies in [c_wob[2], c_mid] + c_tail:
        start(copies)

    for b in range(2):
        @_unrolled_loop(hkv, 8)
        def _(h):
            o = o_s[b * hkv + h] / jnp.sum(l_s[b * hkv + h], axis=1, keepdims=True)
            att[b, :, _ds(h * 2 * DH, 2 * DH, 2 * DH)] = jnp.concatenate(
                [jnp.broadcast_to(o[0:1], (8, DH)), jnp.broadcast_to(o[1:2], (8, DH))], axis=1)

    remaining = iter(range(_N_PRE + 2 * n_k, _N_PIECES))

    def advance(n):
        for _, i in zip(range(n), remaining):
            relay(i)

    early_row0 = 2 * _TAIL_ROWS
    assert d - (_N_PRE + 2 * n_k - lag) // 2 * _W_RUN[0] <= early_row0
    n_low = _WOB_SPLIT * _W_GROUP
    advance(1)
    emit(early_row0, out_proj(0, lambda c: woa[early_row0:, c], jnp.zeros((8, d - early_row0), f32), 0, E))
    advance(2)
    wait(c_wob[0])
    emit(d, out_proj(1, lambda c: wob[low, :, c], jnp.zeros((8, n_low), f32), 0, E))
    advance(1)
    wait(c_wob[1])
    res = out_proj(1, lambda c: wob[high, :, c], jnp.zeros((8, d - n_low), f32), 0, E // 2)
    advance(_N_PIECES)
    wait(c_wob[2])
    emit(d + n_low, out_proj(1, lambda c: wob[high, :, c], res, E // 2, E))
    for i in range(_N_PIECES - lag, _N_PIECES):
        relay_out(i).wait()
    wait(c_mid)
    emit(_TAIL_ROWS, out_dot(0, woa[_TAIL_ROWS:early_row0], pl.ds(0, E)))

    acc_s[...] = jnp.zeros(acc_s.shape, f32)
    for copies, cols in zip(c_tail[:-1], tail_cols):
        wait(copies)
        acc_s[...] = acc_s[...] + out_dot(0, woa[:_TAIL_ROWS, cols], cols)
    wait(c_tail[-1])
    emit(0, acc_s[...] + out_dot(0, woa[:_TAIL_ROWS, tail_cols[-1]], tail_cols[-1]))


@jax.jit
def pallas_concat_heads__gqa_block_cached__sliding_block_cached__decode_kernel(
    A_x: jax.Array,
    A_k_cache: jax.Array,
    A_v_cache: jax.Array,
    A_wq: jax.Array,
    A_wo: jax.Array,
    B_x: jax.Array,
    B_k_cache: jax.Array,
    B_v_cache: jax.Array,
    B_wq: jax.Array,
    B_wo: jax.Array,
):
    _, hkv, sk, _ = A_k_cache.shape
    d = A_x.shape[-1]
    win = min(4096, max(256, sk // 4))
    assert A_x.shape == (1, 1, d) and HQ == 2 * hkv and B_k_cache.shape == A_k_cache.shape
    assert sk % _CHUNK == 0 and win % _CHUNK == 0 and d % _W_GROUP == 0
    n_k = (sk + win) // _CHUNK
    dt, f32 = A_x.dtype, jnp.float32
    grouped = (d // _W_GROUP, _W_GROUP, E)
    cache = (hkv, sk, DH)

    def kernel(*refs):
        pl.run_scoped(
            functools.partial(_body, *refs),
            pltpu.SemaphoreType.DMA((2 * n_k + _N_SEMS,)),
            pltpu.SemaphoreType.DMA((_N_STAGE,)),
            pltpu.SemaphoreType.DMA((_N_STAGE,)),
        )

    out = pl.pallas_call(
        kernel,
        out_shape=jax.ShapeDtypeStruct((1, 2 * d), dt),
        in_specs=[pl.BlockSpec(memory_space=pltpu.HBM)] * 10,
        out_specs=pl.BlockSpec(memory_space=pltpu.VMEM),
        scratch_shapes=[
            pltpu.VMEM((2, 1, d), dt),
            pltpu.VMEM((2,) + grouped, dt),
            pltpu.VMEM((2 * n_k, hkv, _CHUNK, DH), dt),
            pltpu.VMEM((d, E), dt),
            pltpu.VMEM(grouped, dt),
            pltpu.VMEM((2 * hkv, 8, DH), f32),
            pltpu.VMEM((n_k, hkv, 8, _CHUNK), f32),
            pltpu.VMEM((2 * hkv, 8, 128), f32),
            pltpu.VMEM((2 * hkv, 8, 128), f32),
            pltpu.VMEM((2 * hkv, 8, DH), f32),
            pltpu.VMEM((2, 8, E), f32),
            pltpu.VMEM((8, _TAIL_ROWS), f32),
            pltpu.SMEM((_N_STAGE,) + _W_RUN, dt),
        ],
        compiler_params=pltpu.CompilerParams(vmem_limit_bytes=120 * 1024 * 1024),
    )(
        A_x.reshape(1, d), A_k_cache.reshape(cache), A_v_cache.reshape(cache),
        A_wq.reshape(grouped), A_wo.T,
        B_x.reshape(1, d), B_k_cache.reshape(cache), B_v_cache.reshape(cache),
        B_wq.reshape(grouped), B_wo.T.reshape(grouped),
    )
    return out.reshape(1, 1, 2 * d)
```

```python
import functools

import jax
import jax.numpy as jnp
from jax import lax
import jax.experimental.pallas as pl
import jax.experimental.pallas.tpu as pltpu

HQ, DH = 32, 128
E = HQ * DH
_NT = (((1,), (1,)), ((), ()))

_CHUNK = 256
_RUNS = (192, 192, 128)
_LOOKAHEAD = 8
_W_RUN = (8, 2048)
_W_GROUP = 48
_WOB_SPLIT = 7
_N_PIECES = 95
_N_STAGE = 4
_AHEAD = 2
_N_PRE = 11
_TAIL_ROWS = 128
_TAIL_COLS = (2048, 1024, 1024)
_N_SEMS = 9 + len(_TAIL_COLS)


def _ds(start, size, align):
    if not isinstance(start, int):
        start = pl.multiple_of(start, align)
    return pl.ds(start, size)


def _fold(op, acc, x):
    for j in range(x.shape[1] // 128):
        acc = op(acc, x[:, j * 128:(j + 1) * 128])
    return acc


def _unrolled_loop(n, unroll):
    def run(fn):
        @pl.loop(0, n // unroll)
        def _(g):
            for i in range(unroll):
                fn(g * unroll + i)
    return run


def _body(xa_h, ka_h, va_h, wqa_h, woa_h, xb_h, kb_h, vb_h, wqb_h, wob_h, out_ref,
          x_s, wq, kv, woa, wob, q_s, s_s, m_s, l_s, o_s, att, acc_s, stage,
          sems, in_sems, out_sems):
    f32, bf16 = jnp.float32, jnp.bfloat16
    hkv, sk, _ = ka_h.shape
    d = woa.shape[0]
    n_k = kv.shape[0]
    n_a = sk // _CHUNK
    win0 = sk - (n_k - n_a) * _CHUNK
    scale = DH ** -0.5

    next_sem = iter(range(n_k, n_k + _N_SEMS))

    def blocks(src, dst, indices):
        sem = sems.at[next(next_sem)]
        return [pltpu.make_async_copy(src.at[ix], dst.at[ix], sem) for ix in indices]

    def slabs(src, dst, groups, c0, c1):
        return blocks(src, dst, [(groups, pl.ds(r, _W_RUN[0]), pl.ds(c, _W_RUN[1]))
                                 for c in range(c0, c1, _W_RUN[1])
                                 for r in range(0, _W_GROUP, _W_RUN[0])])

    def start(copies):
        for c in copies:
            c.start()

    def wait(copies):
        for c in copies:
            c.wait()

    caches = ((0, n_a, ka_h, 0), (n_a, n_k, kb_h, win0),
              (n_k, n_k + n_a, va_h, 0), (n_k + n_a, 2 * n_k, vb_h, win0))

    def kv_start(j, candidates):
        for lo, hi, src, row0 in candidates:
            @pl.when((j >= lo) & (j < hi) & ((j & 1) == 0))
            def _():
                for i, n in enumerate(_RUNS):
                    r = sum(_RUNS[:i])
                    pltpu.make_async_copy(src.at[:, _ds(row0 + (j - lo) * _CHUNK + r, n, 16)],
                                          kv.at[j >> 1, :, pl.ds(r, n)], sems.at[j >> 1]).start()

    def kv_wait(j):
        @pl.when((j & 1) == 0)
        def _():
            pltpu.make_async_copy(kv.at[j >> 1], kv.at[j >> 1], sems.at[j >> 1]).wait()

    def kv_chunk(j, h):
        return kv[j >> 1, h, _ds((j & 1) * _CHUNK, _CHUNK, _CHUNK)]

    lag = _N_STAGE - _AHEAD

    def piece(i):
        return (_ds(d - _W_RUN[0] - (i >> 1) * _W_RUN[0], _W_RUN[0], _W_RUN[0]),
                _ds((i & 1) * _W_RUN[1], _W_RUN[1], _W_RUN[1]))

    def relay_in(i):
        slot = i & (_N_STAGE - 1)
        return pltpu.make_async_copy(woa_h.at[piece(i)], stage.at[slot], in_sems.at[slot])

    def relay_out(i):
        slot = i & (_N_STAGE - 1)
        return pltpu.make_async_copy(stage.at[slot], woa.at[piece(i)], out_sems.at[slot])

    def relay(i):
        traced = not isinstance(i, int)
        relay_in(i).wait()
        relay_out(i).start()
        if traced or i >= lag:
            relay_out(i - lag).wait()
        if traced or i + _AHEAD < _N_PIECES:
            relay_in(i + _AHEAD).start()

    assert lag <= _N_PRE - _LOOKAHEAD and _N_PRE + 2 * n_k + _AHEAD <= _N_PIECES

    n_groups = d // _W_GROUP
    every, low, high = pl.ds(0, n_groups), pl.ds(0, _WOB_SPLIT), pl.ds(_WOB_SPLIT, n_groups - _WOB_SPLIT)
    c_wqa = slabs(wqa_h, wq.at[0], every, 0, E)
    c_wqb = slabs(wqb_h, wq.at[1], every, 0, E)
    c_x = [pltpu.make_async_copy(src, x_s.at[b], sems.at[next(next_sem)]) for b, src in enumerate((xa_h, xb_h))]
    c_wob = [slabs(wob_h, wob, low, 0, E), slabs(wob_h, wob, high, 0, E // 2), slabs(wob_h, wob, high, E // 2, E)]
    relayed_row0 = d - (_N_PIECES + 1) // 2 * _W_RUN[0]
    c_mid = blocks(woa_h, woa, [piece(_N_PIECES)] * (_N_PIECES % 2)
                   + [pl.ds(_TAIL_ROWS, relayed_row0 - _TAIL_ROWS)])
    tail_cols = [pl.ds(sum(_TAIL_COLS[:i]), n) for i, n in enumerate(_TAIL_COLS)]
    c_tail = [blocks(woa_h, woa, [(pl.ds(0, _TAIL_ROWS), cols)]) for cols in tail_cols]

    def q_proj(b, h0, n):
        x8 = jnp.broadcast_to(x_s[b], (8, d))
        row = lax.broadcasted_iota(jnp.int32, (8, DH), 0)

        @_unrolled_loop(n, 2)
        def _(i):
            h = h0 + i
            w = wq[b, :, :, _ds(h * 2 * DH, 2 * DH, 2 * DH)].reshape(d, 2 * DH)
            q = jnp.dot(x8, w, preferred_element_type=f32)
            q_s[b * hkv + h] = jnp.where(row == 0, q[:, :DH], q[:, DH:])

    def out_dot(b, w, cols):
        return lax.dot_general(att[b, :, cols].astype(bf16), w, _NT, preferred_element_type=f32)

    def out_proj(b, weights, acc, c0, c1, step=1024):
        def add(i, acc):
            cols = _ds(c0 + i * step, step, step)
            return acc + out_dot(b, weights(cols).reshape(acc.shape[1], step), cols)
        return lax.fori_loop(0, (c1 - c0) // step, add, acc)

    def emit(lane0, res):
        out_ref[:, lane0:lane0 + res.shape[1]] = res[0:1].astype(out_ref.dtype)

    start(c_wqa)
    for i in range(_AHEAD):
        relay_in(i).start()
    start(c_x)
    for i in range(lag):
        relay(i)
    start(c_wqb)
    m_s[...] = jnp.full(m_s.shape, -jnp.inf, f32)
    l_s[...] = jnp.zeros(l_s.shape, f32)
    o_s[...] = jnp.zeros(o_s.shape, f32)

    @pl.loop(lag, _N_PRE)
    def _(i):
        relay(i)
        kv_start(i + _LOOKAHEAD - _N_PRE, caches[:1])

        @pl.when(i == _N_PRE - 2)
        def _():
            wait(c_wqa)
            wait(c_x)

        @pl.when(i >= _N_PRE - 2)
        def _():
            q_proj(0, (i - _N_PRE + 2) * (hkv // 2), hkv // 2)

    @pl.loop(0, n_k)
    def _(j):
        kv_start(j + _LOOKAHEAD, caches[:3])
        relay(_N_PRE + j)

        @pl.when(j == 0)
        def _():
            wait(c_wqb)

        @pl.when(j < 2)
        def _():
            q_proj(1, j * (hkv // 2), hkv // 2)

        kv_wait(j)
        base = jnp.where(j < n_a, 0, hkv)

        @_unrolled_loop(hkv, 8)
        def _(h):
            s = lax.dot_general(q_s[base + h].astype(bf16), kv_chunk(j, h), _NT, preferred_element_type=f32) * scale
            s_s[j, h] = s
            m_s[base + h] = _fold(jnp.maximum, m_s[base + h], s)

    @_unrolled_loop(2 * hkv, 16)
    def _(i):
        m_s[i] = jnp.broadcast_to(jnp.max(m_s[i], axis=1, keepdims=True), (8, 128))

    @pl.loop(0, n_k)
    def _(j):
        kv_start(n_k + j + _LOOKAHEAD, caches[2:])

        @pl.when(j == n_k - 5)
        def _():
            start(c_wob[0])

        @pl.when(j == n_k - 2)
        def _():
            start(c_wob[1])

        relay(_N_PRE + n_k + j)
        kv_wait(n_k + j)
        base = jnp.where(j < n_a, 0, hkv)

        @_unrolled_loop(hkv, 8)
        def _(h):
            p = jnp.exp(s_s[j, h] - jnp.concatenate([m_s[base + h]] * (_CHUNK // 128), axis=1))
            l_s[base + h] = _fold(jnp.add, l_s[base + h], p)
            o_s[base + h] = o_s[base + h] + jnp.dot(p.astype(bf16), kv_chunk(n_k + j, h), preferred_element_type=f32)

    for copies in [c_wob[2], c_mid] + c_tail:
        start(copies)

    for b in range(2):
        @_unrolled_loop(hkv, 8)
        def _(h):
            o = o_s[b * hkv + h] / jnp.sum(l_s[b * hkv + h], axis=1, keepdims=True)
            att[b, :, _ds(h * 2 * DH, 2 * DH, 2 * DH)] = jnp.concatenate(
                [jnp.broadcast_to(o[0:1], (8, DH)), jnp.broadcast_to(o[1:2], (8, DH))], axis=1)

    remaining = iter(range(_N_PRE + 2 * n_k, _N_PIECES))

    def advance(n):
        for _, i in zip(range(n), remaining):
            relay(i)

    early_row0 = 2 * _TAIL_ROWS
    assert d - (_N_PRE + 2 * n_k - lag) // 2 * _W_RUN[0] <= early_row0
    n_low = _WOB_SPLIT * _W_GROUP
    advance(1)
    emit(early_row0, out_proj(0, lambda c: woa[early_row0:, c], jnp.zeros((8, d - early_row0), f32), 0, E))
    advance(1)
    wait(c_wob[0])
    emit(d, out_proj(1, lambda c: wob[low, :, c], jnp.zeros((8, n_low), f32), 0, E))
    advance(1)
    wait(c_wob[1])
    res = out_proj(1, lambda c: wob[high, :, c], jnp.zeros((8, d - n_low), f32), 0, E // 2)
    advance(_N_PIECES)
    wait(c_wob[2])
    emit(d + n_low, out_proj(1, lambda c: wob[high, :, c], res, E // 2, E))
    for i in range(_N_PIECES - lag, _N_PIECES):
        relay_out(i).wait()
    wait(c_mid)
    emit(_TAIL_ROWS, out_dot(0, woa[_TAIL_ROWS:early_row0], pl.ds(0, E)))

    acc_s[...] = jnp.zeros(acc_s.shape, f32)
    for copies, cols in zip(c_tail[:-1], tail_cols):
        wait(copies)
        acc_s[...] = acc_s[...] + out_dot(0, woa[:_TAIL_ROWS, cols], cols)
    wait(c_tail[-1])
    emit(0, acc_s[...] + out_dot(0, woa[:_TAIL_ROWS, tail_cols[-1]], tail_cols[-1]))


@jax.jit
def pallas_concat_heads__gqa_block_cached__sliding_block_cached__decode_kernel(
    A_x: jax.Array,
    A_k_cache: jax.Array,
    A_v_cache: jax.Array,
    A_wq: jax.Array,
    A_wo: jax.Array,
    B_x: jax.Array,
    B_k_cache: jax.Array,
    B_v_cache: jax.Array,
    B_wq: jax.Array,
    B_wo: jax.Array,
):
    _, hkv, sk, _ = A_k_cache.shape
    d = A_x.shape[-1]
    win = min(4096, max(256, sk // 4))
    assert A_x.shape == (1, 1, d) and HQ == 2 * hkv and B_k_cache.shape == A_k_cache.shape
    assert sum(_RUNS) == 2 * _CHUNK and sum(_TAIL_COLS) == E
    assert sk % sum(_RUNS) == 0 and win % sum(_RUNS) == 0 and d % _W_GROUP == 0
    n_k = (sk + win) // _CHUNK
    dt, f32 = A_x.dtype, jnp.float32
    grouped = (d // _W_GROUP, _W_GROUP, E)
    cache = (hkv, sk, DH)

    def kernel(*refs):
        pl.run_scoped(
            functools.partial(_body, *refs),
            pltpu.SemaphoreType.DMA((n_k + _N_SEMS,)),
            pltpu.SemaphoreType.DMA((_N_STAGE,)),
            pltpu.SemaphoreType.DMA((_N_STAGE,)),
        )

    out = pl.pallas_call(
        kernel,
        out_shape=jax.ShapeDtypeStruct((1, 2 * d), dt),
        in_specs=[pl.BlockSpec(memory_space=pltpu.HBM)] * 10,
        out_specs=pl.BlockSpec(memory_space=pltpu.VMEM),
        scratch_shapes=[
            pltpu.VMEM((2, 1, d), dt),
            pltpu.VMEM((2,) + grouped, dt),
            pltpu.VMEM((n_k, hkv, 2 * _CHUNK, DH), dt),
            pltpu.VMEM((d, E), dt),
            pltpu.VMEM(grouped, dt),
            pltpu.VMEM((2 * hkv, 8, DH), f32),
            pltpu.VMEM((n_k, hkv, 8, _CHUNK), f32),
            pltpu.VMEM((2 * hkv, 8, 128), f32),
            pltpu.VMEM((2 * hkv, 8, 128), f32),
            pltpu.VMEM((2 * hkv, 8, DH), f32),
            pltpu.VMEM((2, 8, E), f32),
            pltpu.VMEM((8, _TAIL_ROWS), f32),
            pltpu.SMEM((_N_STAGE,) + _W_RUN, dt),
        ],
        compiler_params=pltpu.CompilerParams(vmem_limit_bytes=120 * 1024 * 1024),
    )(
        A_x.reshape(1, d), A_k_cache.reshape(cache), A_v_cache.reshape(cache),
        A_wq.reshape(grouped), A_wo.T,
        B_x.reshape(1, d), B_k_cache.reshape(cache), B_v_cache.reshape(cache),
        B_wq.reshape(grouped), B_wo.T.reshape(grouped),
    )
    return out.reshape(1, 1, 2 * d)
```
